```python
import os as _os
_os.environ.setdefault("JAX_PLATFORMS", "cpu")
import jax
import jax.numpy as jnp

def _softmax(x, axis=-1):
    return jax.nn.softmax(x, axis=axis)
def _gelu(x):
    return jax.nn.gelu(x, approximate=True)
def _silu(x):
    return jax.nn.silu(x)
def _sigmoid(x):
    return jax.nn.sigmoid(x)
def _layernorm(x, axis=-1, eps=1e-5):
    m = jnp.mean(x, axis=axis, keepdims=True)
    v = jnp.var(x, axis=axis, keepdims=True)
    return (x - m) / jnp.sqrt(v + eps)
def _scatter_add(tgt, idx, src, axis=0):
    return tgt.at[idx].add(src)
def _segment_sum(src, seg, n):
    return jax.ops.segment_sum(src, seg, n)
class _Rng:
    def __init__(self, key):
        self._k = key
    def _next(self):
        self._k, sub = jax.random.split(self._k)
        return sub
    def normal(self, shape):
        return jax.random.normal(self._next(), shape, dtype=jnp.bfloat16)
    def randint(self, lo, hi, shape):
        return jax.random.randint(self._next(), shape, lo, hi, dtype=jnp.int32)
    def uniform(self, shape, lo=0.0, hi=1.0):
        return jax.random.uniform(self._next(), shape, jnp.bfloat16, lo, hi)
    def permutation(self, n):
        return jax.random.permutation(self._next(), n)


kernel_name = 'standalone__gqa_block_cached__near_ridge'

def setup_inputs():
    _rng = _Rng(jax.random.key(int.from_bytes(__import__("os").urandom(4), "little")))
    _w = (lambda a: (lambda t: t.astype(jnp.bfloat16) if jnp.issubdtype(t.dtype, jnp.floating) else t)(jnp.asarray(a)))
    B, Sq, D = 16, 96, 576
    Hq, Hkv, Sk, Dh = 32, 16, 512, 128
    assert Hq % Hkv == 0, (Hq, Hkv)
    return {
        "x": _w((lambda *s: _rng.normal(s) * 0.2)(B, Sq, D)),
        "k_cache": _w((lambda *s: _rng.normal(s) * 3.2)(B, Hkv, Sk, Dh)),
        "v_cache": _w((lambda *s: _rng.normal(s) * 0.05)(B, Hkv, Sk, Dh)),
        "wq": _w((lambda *s: _rng.normal(s) * 0.2)(D, Hq * Dh) * (D ** -0.5)),
        "wo": _w((lambda *s: _rng.normal(s) * 0.05)(Hq * Dh, D) * ((Hq * Dh) ** -0.5)),
    }

def reference(x, k_cache, v_cache, wq, wo):
    B, Sq, D = x.shape
    Hq, Dh = 32, 128
    Hkv = k_cache.shape[1]
    rep = Hq // Hkv
    q = (lambda x, *d: x.transpose(*d))((x @ wq).reshape(B, Sq, Hq, Dh), 0, 2, 1, 3)
    k = jnp.repeat(k_cache, rep, axis=1)
    v = jnp.repeat(v_cache, rep, axis=1)
    scores = jnp.einsum("bhqd,bhkd->bhqk", q, k) * (Dh ** -0.5)
    p = _softmax(scores, axis=-1)
    o = jnp.einsum("bhqk,bhkd->bhqd", p, v)
    return (lambda x, *d: x.transpose(*d))(o, 0, 2, 1, 3).reshape(B, Sq, Hq * Dh) @ wo
```

```python
import functools
import jax
import jax.numpy as jnp
import jax.experimental.pallas as pl
import jax.experimental.pallas.tpu as pltpu

LOG2E = 1.4426950408889634
NT = (((1,), (1,)), ((), ()))

def make(vmem=100, CB=4, newton=True):
    @jax.jit
    def f(x, k_cache, v_cache, wq, wo):
        B, Sq, D = x.shape
        _, Hkv, Sk, Dh = k_cache.shape
        Hq = wq.shape[1] // Dh
        rep = Hq // Hkv
        scale = (Dh ** -0.5) * LOG2E
        M = B * Sq
        W = rep * Dh
        NC = B // CB
        CM = CB * Sq
        x2 = x.reshape(B * Sq, D)
        woT = wo.T

        def kern(x_ref, k_ref, v_ref, wq_ref, woT_ref, o_ref, acc_ref):
            h = pl.program_id(0)

            @pl.when(h == 0)
            def _():
                acc_ref[...] = jnp.zeros_like(acc_ref)

            qs, ss, os = {}, {}, {}
            def Q(c):
                q = jnp.dot(x_ref[c * CM:(c + 1) * CM, :], wq_ref[...], preferred_element_type=jnp.float32)
                qs[c] = (q * scale).astype(jnp.bfloat16)
            def QK(u):
                c, g = divmod(u, CB)
                qg = qs[c][g * Sq:(g + 1) * Sq]
                qq = jnp.concatenate([qg[:, r * Dh:(r + 1) * Dh] for r in range(rep)], axis=0)
                ss[u] = jax.lax.dot_general(qq, k_ref[u, 0], NT, preferred_element_type=jnp.float32)
            def PV(u):
                s = ss.pop(u)
                m = jnp.max(s, axis=-1, keepdims=True)
                p = jnp.exp2(s - m)
                l = jnp.sum(p, axis=-1, keepdims=True)
                o = jnp.dot(p.astype(jnp.bfloat16), v_ref[u, 0], preferred_element_type=jnp.float32)
                r = pl.reciprocal(l, approx=True)
                if newton:
                    r = r * (2.0 - l * r)
                o = (o * r).astype(jnp.bfloat16)
                os[u] = jnp.concatenate([o[r * Sq:(r + 1) * Sq] for r in range(rep)], axis=1)
            def O(c):
                o = jnp.concatenate([os.pop(c * CB + g) for g in range(CB)], axis=0)
                y = jax.lax.dot_general(woT_ref[...], o, NT, preferred_element_type=jnp.float32)
                acc_ref[:, c * CM:(c + 1) * CM] += y

            Q(0); Q(1); QK(0)
            for u in range(B):
                if u + 1 < B:
                    QK(u + 1)
                PV(u)
                c, g = divmod(u, CB)
                if g == CB - 2 and c + 2 < NC:
                    Q(c + 2)
                if g == 0 and 1 <= c < NC - 1:
                    O(c - 1)
            O(NC - 2); O(NC - 1)

            @pl.when(h == Hkv - 1)
            def _():
                o_ref[...] = acc_ref[...].T.astype(o_ref.dtype)

        out = pl.pallas_call(
            kern,
            grid=(Hkv,),
            in_specs=[
                pl.BlockSpec((M, D), lambda h: (0, 0)),
                pl.BlockSpec((B, 1, Sk, Dh), lambda h: (0, h, 0, 0)),
                pl.BlockSpec((B, 1, Sk, Dh), lambda h: (0, h, 0, 0)),
                pl.BlockSpec((D, W), lambda h: (0, h)),
                pl.BlockSpec((D, W), lambda h: (0, h)),
            ],
            out_specs=pl.BlockSpec((M, D), lambda h: (0, 0)),
            out_shape=jax.ShapeDtypeStruct((B * Sq, D), x.dtype),
            scratch_shapes=[pltpu.VMEM((D, M), jnp.float32)],
            compiler_params=pltpu.CompilerParams(
                dimension_semantics=("arbitrary",),
                vmem_limit_bytes=vmem * 1024 * 1024),
        )(x2, k_cache, v_cache, wq, woT)
        return out.reshape(B, Sq, D)
    return f

pallas_standalone__gqa_block_cached__near_ridge_kernel = make()
```

```python
import contextlib
import jax
import jax.numpy as jnp
import jax.experimental.pallas as pl
import jax.experimental.pallas.tpu as pltpu

LOG2E = 1.4426950408889634
NT = (((1,), (1,)), ((), ()))

def make(vmem=100, newton=True, scopes=False, bp=1, qsplit=2, osplit=2, lastbar=True, bc=True):
    sc_ = (lambda n: jax.named_scope(n)) if scopes else (lambda n: contextlib.nullcontext())
    CB, LA, NB = 4, 4, 8
    @jax.jit
    def f(x, k_cache, v_cache, wq, wo):
        B, Sq, D = x.shape
        _, Hkv, Sk, Dh = k_cache.shape
        Hq = wq.shape[1] // Dh
        rep = Hq // Hkv
        scale = (Dh ** -0.5) * LOG2E
        M = B * Sq
        W = rep * Dh
        NC = B // CB
        CM = CB * Sq
        x2 = x.reshape(B * Sq, D)
        woT = wo.T
        T = 128
        H0 = Hkv - LA

        def kern(x_hbm, k_hbm, v_hbm, wq_hbm, woT_hbm, o_hbm,
                 x_ref, kvbuf, wq0buf, wbuf, q_ref, acc_ref, cur_ref, fin_ref, obuf,
                 xsem, kvsem, wq0sem, wsem, osem):
            def slot(h):
                return h % NB if isinstance(h, int) else jnp.bitwise_and(h, NB - 1)
            def col(h):
                return h * W if isinstance(h, int) else pl.multiple_of(h * W, W)
            def x_cp(c):
                return pltpu.make_async_copy(x_hbm.at[pl.ds(c * CM, CM)], x_ref.at[pl.ds(c * CM, CM)], xsem.at[c])
            def wq0_cp(h):
                return pltpu.make_async_copy(wq_hbm.at[:, pl.ds(col(h), W)], wq0buf.at[h], wq0sem.at[h])
            def start_kv(h):
                s = slot(h)
                pltpu.make_async_copy(k_hbm.at[:, h], kvbuf.at[s, 0], kvsem.at[s]).start(priority=bp)
                pltpu.make_async_copy(v_hbm.at[:, h], kvbuf.at[s, 1], kvsem.at[s]).start(priority=bp)
            def start_w(h):
                s = slot(h)
                hq = min(h + LA, Hkv - 1) if isinstance(h, int) else jnp.minimum(h + LA, Hkv - 1)
                pltpu.make_async_copy(wq_hbm.at[:, pl.ds(col(hq), W)], wbuf.at[s, 0], wsem.at[s]).start(priority=bp)
                pltpu.make_async_copy(woT_hbm.at[:, pl.ds(col(h), W)], wbuf.at[s, 1], wsem.at[s]).start(priority=bp)
            def start_head(h):
                start_w(h); start_kv(h)
            def wait_head(h):
                s = slot(h)
                pltpu.make_async_copy(kvbuf.at[s], kvbuf.at[s], kvsem.at[s]).wait()
                pltpu.make_async_copy(wbuf.at[s], wbuf.at[s], wsem.at[s]).wait()
            def o_cp(c, t0, n, i):
                r0 = c * CM + t0
                if not isinstance(r0, int):
                    r0 = pl.multiple_of(r0, 16)
                return pltpu.make_async_copy(obuf.at[c, pl.ds(t0, n)], o_hbm.at[pl.ds(r0, n)], osem.at[i])

            def Q(h, c, w_ref, nsplit):
                s = slot(h)
                gb = CB // nsplit
                for j in range(nsplit):
                    b0 = c * CB + j * gb
                    q = jnp.dot(x_ref[b0 * Sq:(b0 + gb) * Sq, :], w_ref[...], preferred_element_type=jnp.float32)
                    q = (q * scale).astype(jnp.bfloat16)
                    for g in range(gb):
                        for r in range(rep):
                            q_ref[s, b0 + g, r * Sq:(r + 1) * Sq, :] = q[g * Sq:(g + 1) * Sq, r * Dh:(r + 1) * Dh]

            if bc:
                kv32 = kvbuf.bitcast(jnp.uint32)
                q32 = q_ref.bitcast(jnp.uint32)
                ld_kv = lambda s, i, b: pltpu.bitcast(kv32[s, i, b], jnp.bfloat16)
                ld_q = lambda s, b: pltpu.bitcast(q32[s, b], jnp.bfloat16)
            else:
                ld_kv = lambda s, i, b: kvbuf[s, i, b]
                ld_q = lambda s, b: q_ref[s, b]
            def qk(q, s, b):
                return jax.lax.dot_general(q, ld_kv(s, 0, b), NT, preferred_element_type=jnp.float32)
            def sm(sc):
                m = jnp.max(sc, axis=-1, keepdims=True)
                p = jnp.exp2(sc - m)
                l = jnp.sum(p, axis=-1, keepdims=True)
                return p.astype(jnp.bfloat16), l
            def pv(sc, s, b):
                p, l = sc if isinstance(sc, tuple) else sm(sc)
                o = jnp.dot(p, ld_kv(s, 1, b), preferred_element_type=jnp.float32)
                r = pl.reciprocal(l, approx=True)
                if newton:
                    r = r * (2.0 - l * r)
                o = (o * r).astype(jnp.bfloat16)
                return jnp.concatenate([o[r * Sq:(r + 1) * Sq] for r in range(rep)], axis=1)
            def oproj(wo_refs, o, msplit):
                dm = D // msplit
                ys = []
                for j in range(msplit):
                    w = [r[j * dm:(j + 1) * dm, :] for r in wo_refs]
                    w = jnp.concatenate(w, axis=1) if len(w) > 1 else w[0]
                    ys.append(jax.lax.dot_general(w, o, NT, preferred_element_type=jnp.float32))
                return jnp.concatenate(ys, axis=0) if msplit > 1 else ys[0]

            def main_body(h):
                s = slot(h)
                ss, os = {}, {}
                qpre = {u: ld_q(s, u) for u in range(2)}
                def QK(u):
                    ss[u] = qk(qpre[u] if u in qpre else ld_q(s, u), s, u)
                def PV(u):
                    os[u] = pv(ss.pop(u), s, u)
                def O(c):
                    o = jnp.concatenate([os.pop(c * CB + g) for g in range(CB)], axis=0)
                    acc_ref[c] += oproj([wbuf.at[s, 1]], o, osplit)
                def QQ(c):
                    Q(h + LA, c, wbuf.at[s, 0], qsplit)
                start_kv(h + LA)
                QQ(0)
                start_w(h + LA)
                QK(0)
                for u in range(B):
                    if u + 1 < B:
                        QK(u + 1)
                    c, g = divmod(u, CB)
                    if g == 0 and 1 <= c < NC - 1:
                        QQ(c)
                    if g == 1 and c >= 1:
                        O(c - 1)
                    PV(u)
                QQ(NC - 1)
                O(NC - 1)

            def emit_out(c, t0, n, y):
                obuf[c, t0:t0 + n, :] = y.T.astype(obuf.dtype)

            def tail_body(c):
                units = [(hh, g) for hh in range(LA) for g in range(CB)]
                ss, os = {}, {}
                def QK(i):
                    hh, g = units[i]
                    s = slot(H0 + hh)
                    ss[i] = qk(ld_q(s, c * CB + g), s, c * CB + g)
                def PV(i):
                    hh, g = units[i]
                    os[i] = pv(ss.pop(i), slot(H0 + hh), c * CB + g)
                def O(hhs):
                    o = jnp.concatenate([jnp.concatenate([os.pop(hh * CB + g) for g in range(CB)], axis=0) for hh in hhs], axis=1)
                    y = oproj([wbuf.at[slot(H0 + hh), 1] for hh in hhs], o, osplit if len(hhs) == 1 else 1)
                    src = acc_ref.at[c] if hhs[0] == 0 else cur_ref
                    dst = fin_ref if hhs[-1] == LA - 1 else cur_ref
                    dst[...] = src[...] + y
                cp_ = jnp.bitwise_and(c + NC - 1, NC - 1)
                emit_out(cp_, 0, CM, fin_ref[...])
                @pl.when(c > 0)
                def _():
                    o_cp(cp_, 0, CM, cp_).start()
                QK(0)
                n = len(units)
                for i in range(n):
                    if i + 1 < n:
                        QK(i + 1)
                    if i % CB == 1 and 1 <= i // CB <= LA - 2:
                        O([i // CB - 1])
                    PV(i)
                O([LA - 2]); O([LA - 1])

            def last_body(c):
                units = [(hh, g) for g in range(CB) for hh in range(LA)]
                ss, os = {}, {}
                outs = []
                def QK(i):
                    hh, g = units[i]
                    s = slot(H0 + hh)
                    ss[i] = qk(ld_q(s, c * CB + g), s, c * CB + g)
                def PV(i):
                    hh, g = units[i]
                    os[units[i]] = pv(ss.pop(i), slot(H0 + hh), c * CB + g)
                def rows(hh, t0, n):
                    parts = []
                    for g in range(t0 // Sq, (t0 + n - 1) // Sq + 1):
                        a, b = max(t0, g * Sq), min(t0 + n, (g + 1) * Sq)
                        parts.append(os[(hh, g)][a - g * Sq:b - g * Sq])
                    return jnp.concatenate(parts, axis=0) if len(parts) > 1 else parts[0]
                def Opart(t0, hhs):
                    o = jnp.concatenate([rows(hh, t0, T) for hh in hhs], axis=1)
                    return oproj([wbuf.at[slot(H0 + hh), 1] for hh in hhs], o, 1)
                def piece(j):
                    t0 = j * T
                    y = acc_ref[c, :, t0:t0 + T] + Opart(t0, [0, 1])
                    y = y + Opart(t0, [2, 3])
                    emit_out(c, t0, T, y)
                    cp = o_cp(c, t0, T, NC - 1 + j)
                    cp.start(); outs.append(cp)
                emit_out(c - 1, 0, CM, fin_ref[...])
                o_cp(c - 1, 0, CM, c - 1).start()
                QK(0)
                n = len(units)
                for i in range(n):
                    if i + 1 < n:
                        QK(i + 1)
                    if i == 2 * LA + 1:
                        piece(0)
                    if i == 3 * LA + 1:
                        piece(1)
                    if lastbar and i == n - 2:
                        ss[i] = sm(ss[i])
                        o_cp(0, 0, CM, 0).wait()
                    PV(i)
                piece(2)
                with sc_('outw'):
                    for cc in range(NC - 1):
                        if not (lastbar and cc == 0):
                            o_cp(cc, 0, CM, cc).wait()
                    for cp in outs:
                        cp.wait()

            x_cp(0).start(); wq0_cp(0).start(); wq0_cp(1).start(); x_cp(1).start()
            wq0_cp(2).start(); wq0_cp(3).start(); x_cp(2).start(); x_cp(3).start()
            for hh in range(LA):
                start_head(hh)
            with sc_('zero'):
                acc_ref[...] = jnp.zeros_like(acc_ref)
                fin_ref[...] = jnp.zeros_like(fin_ref)
            with sc_('w0'):
                x_cp(0).wait(); wq0_cp(0).wait()
            with sc_('p0'):
                Q(0, 0, wq0buf.at[0], 2)
            with sc_('w1'):
                wq0_cp(1).wait()
            with sc_('p1'):
                Q(1, 0, wq0buf.at[1], 2)
            with sc_('w2'):
                x_cp(1).wait(); wq0_cp(2).wait()
            with sc_('p2'):
                Q(0, 1, wq0buf.at[0], 1); Q(1, 1, wq0buf.at[1], 1)
                Q(2, 0, wq0buf.at[2], 1); Q(2, 1, wq0buf.at[2], 1)
            with sc_('w3'):
                wq0_cp(3).wait(); x_cp(2).wait(); x_cp(3).wait()
            with sc_('p3'):
                Q(3, 0, wq0buf.at[3], 1); Q(3, 1, wq0buf.at[3], 1)
                for c in range(2, NC):
                    for hh in range(LA):
                        Q(hh, c, wq0buf.at[hh], 1)

            def loop_main(h, carry):
                with sc_('wait'):
                    wait_head(h)
                with sc_('body'):
                    main_body(h)
                return carry
            jax.lax.fori_loop(0, H0, loop_main, 0)
            with sc_('wait'):
                for hh in range(LA):
                    wait_head(H0 + hh)
            def loop_tail(c, carry):
                with sc_('tail'):
                    tail_body(c)
                return carry
            jax.lax.fori_loop(0, NC - 1, loop_tail, 0)
            with sc_('last'):
                last_body(NC - 1)

        ms = pltpu.HBM
        out = pl.pallas_call(
            kern,
            in_specs=[pl.BlockSpec(memory_space=ms)] * 5,
            out_specs=pl.BlockSpec(memory_space=ms),
            out_shape=jax.ShapeDtypeStruct((B * Sq, D), x.dtype),
            scratch_shapes=[
                pltpu.VMEM((M, D), x.dtype),
                pltpu.VMEM((NB, 2, B, Sk, Dh), x.dtype),
                pltpu.VMEM((LA, D, W), x.dtype),
                pltpu.VMEM((NB, 2, D, W), x.dtype),
                pltpu.VMEM((NB, B, rep * Sq, Dh), x.dtype),
                pltpu.VMEM((NC, D, CM), jnp.float32),
                pltpu.VMEM((D, CM), jnp.float32),
                pltpu.VMEM((D, CM), jnp.float32),
                pltpu.VMEM((NC, CM, D), x.dtype),
                pltpu.SemaphoreType.DMA((NC,)),
                pltpu.SemaphoreType.DMA((NB,)),
                pltpu.SemaphoreType.DMA((LA,)),
                pltpu.SemaphoreType.DMA((NB,)),
                pltpu.SemaphoreType.DMA((NC - 1 + CM // T,)),
            ],
            compiler_params=pltpu.CompilerParams(
                vmem_limit_bytes=vmem * 1024 * 1024, disable_bounds_checks=True),
        )(x2, k_cache, v_cache, wq, woT)
        return out.reshape(B, Sq, D)
    return f

pallas_standalone__gqa_block_cached__near_ridge_kernel = make()
```

```python
import contextlib
import jax
import jax.numpy as jnp
import jax.experimental.pallas as pl
import jax.experimental.pallas.tpu as pltpu

LOG2E = 1.4426950408889634
NT = (((1,), (1,)), ((), ()))
CA = [[(0, 0, 1), (1, 1, 1)], [(1, 0, 1), (1, 1, 1)], [(0, 0, 1)], [(1, 1, 1)],
      [(0, 0, 1), (0, 1, 1)], [(1, 0, 1), (0, 0, -1)], [(0, 1, 1), (1, 1, -1)]]
CBm = [[(0, 0, 1), (1, 1, 1)], [(0, 0, 1)], [(0, 1, 1), (1, 1, -1)], [(1, 0, 1), (0, 0, -1)],
       [(1, 1, 1)], [(0, 0, 1), (0, 1, 1)], [(1, 0, 1), (1, 1, 1)]]
CC = [[[(0, 1), (3, 1), (6, 1), (4, -1)], [(2, 1), (4, 1)]], [[(1, 1), (3, 1)], [(0, 1), (2, 1), (5, 1), (1, -1)]]]


def lin(terms):
    acc = terms[0][0]()
    for th, sg in terms[1:]:
        acc = acc + th() if sg > 0 else acc - th()
    return acc


def diag(terms):
    return [terms[0], terms[3], terms[1], terms[2]] if len(terms) == 4 else terms


def memo(fn):
    cache = {}
    def g(*a):
        if a not in cache:
            cache[a] = fn(*a)
        return cache[a]
    return g


def zero_bits(tok):
    u = pltpu.bitcast(tok, jnp.uint32)
    return jax.lax.shift_right_logical(jax.lax.shift_right_logical(u, jnp.uint32(31)), jnp.uint32(1))


def make(vmem=100, newton=True, scopes=False, bp=1, qsplit=2,
         qpos=((5, 11), (8, 12)), opos=(8, 12), apos=(1, 3, 5, 7), acap=3, splan=(10, 6, 0, 0),
         tsp=6, g0pos=None, g1pos=None, c0start=45, midbar=None, cdl=8, pdl=(58, 62, ('O', 3, 2)), c1dl=(58, 59, 62, 63), bpin=2, boff=(2, 4), bstart=0, ostage=True, bulkat=0, bp0=1):
    sc_ = (lambda n: jax.named_scope(n)) if scopes else (lambda n: contextlib.nullcontext())
    CB, LA, NB, T, RG = 4, 4, 8, 128, 16
    bf = lambda a: a.astype(jnp.bfloat16)

    @jax.jit
    def f(x, k_cache, v_cache, wq, wo):
        B, Sq, D = x.shape
        _, Hkv, Sk, Dh = k_cache.shape
        Hq = wq.shape[1] // Dh
        rep = Hq // Hkv
        scale = (Dh ** -0.5) * LOG2E
        M = B * Sq
        W = rep * Dh
        NC = B // CB
        CM = CB * Sq
        DQ = D // 4
        NT3 = CM // T
        H0 = Hkv - LA
        NTL = M // T
        x2 = x.reshape(M, D)
        woT = wo.T

        def kern(x_hbm, k_hbm, v_hbm, wq_hbm, woT_hbm, o_hbm,
                 x_ref, kvbuf, wq0buf, wqbuf, wobuf, q_ref, sbuf, macc, base, oscr, obuf, zs,
                 sems):
            class _S:
                def __init__(self, off):
                    self.off = off
                    self.at = self
                def __getitem__(self, i):
                    return sems.at[self.off + i]
            xsem, kvsem, wq0sem, wqsem, wosem, osem = [_S(o) for o in (0, 8, 16, 24, 32, 40)]
            kv32 = kvbuf.bitcast(jnp.uint32)
            q32 = q_ref.bitcast(jnp.uint32)
            s32 = sbuf.bitcast(jnp.uint32)

            def slot(h):
                return h % NB if isinstance(h, int) else jnp.bitwise_and(h, NB - 1)
            def col(h):
                return h * W if isinstance(h, int) else pl.multiple_of(h * W, W)
            def x_cp(c):
                r0 = c * CM if isinstance(c, int) else pl.multiple_of(c * CM, CM)
                return pltpu.make_async_copy(x_hbm.at[pl.ds(r0, CM)], x_ref.at[pl.ds(r0, CM)], xsem.at[c])
            def wq0_cp(h):
                return pltpu.make_async_copy(wq_hbm.at[:, pl.ds(col(h), W)], wq0buf.at[h], wq0sem.at[h])
            def start_kv(h, p=bp):
                s = slot(h)
                pltpu.make_async_copy(k_hbm.at[:, h], kvbuf.at[s, 0], kvsem.at[s]).start(priority=p)
                pltpu.make_async_copy(v_hbm.at[:, h], kvbuf.at[s, 1], kvsem.at[s]).start(priority=p)
            def wait_kv(h):
                s = slot(h)
                pltpu.make_async_copy(kvbuf.at[s], kvbuf.at[s], kvsem.at[s]).wait()
            def wq_cp(h):
                hq = min(h + LA, Hkv - 1) if isinstance(h, int) else jnp.minimum(h + LA, Hkv - 1)
                return pltpu.make_async_copy(wq_hbm.at[:, pl.ds(col(hq), W)], wqbuf.at[slot(h)], wqsem.at[slot(h)])
            def wo_cp(h):
                return pltpu.make_async_copy(woT_hbm.at[:, pl.ds(col(h), W)], wobuf.at[slot(h)], wosem.at[slot(h)])
            def o_cp(tile):
                return pltpu.make_async_copy(obuf.at[tile], o_hbm.at[pl.ds(tile * T, T)], osem.at[tile])

            def Qb(h, b0, gb, w_ref):
                s = slot(h)
                toks = []
                for r in range(rep):
                    r0 = b0 * Sq if isinstance(b0, int) else pl.multiple_of(b0 * Sq, Sq)
                    q = jnp.dot(x_ref[pl.ds(r0, gb * Sq), :], w_ref[:, r * Dh:(r + 1) * Dh], preferred_element_type=jnp.float32)
                    toks.append(q)
                    q = bf(q * scale)
                    for g in range(gb):
                        q_ref[s, b0 + g, r * Sq:(r + 1) * Sq, :] = q[g * Sq:(g + 1) * Sq]
                return toks

            ld_kv = lambda s, i, b: pltpu.bitcast(kv32[s, i, b], jnp.bfloat16)
            ld_q = lambda s, b: pltpu.bitcast(q32[s, b], jnp.bfloat16)
            def qk(q, s, b):
                return jax.lax.dot_general(q, ld_kv(s, 0, b), NT, preferred_element_type=jnp.float32)
            def sm(sc):
                m = jnp.max(sc, axis=-1, keepdims=True)
                p = jnp.exp2(sc - m)
                pt = [p[:, t * T:(t + 1) * T] for t in range(Sk // T)]
                ps = pt[0]
                for t in range(1, Sk // T):
                    ps = ps + pt[t]
                pt[-1] = jnp.minimum(pt[-1], ps)
                return bf(jnp.concatenate(pt, axis=1)), jnp.sum(ps, axis=-1, keepdims=True)
            def pv(sc, s, b):
                p, l = sc if isinstance(sc, tuple) else sm(sc)
                o = jnp.dot(p, ld_kv(s, 1, b), preferred_element_type=jnp.float32)
                r = pl.reciprocal(l, approx=True)
                if newton:
                    r = r * (2.0 - l * r)
                return o * r, o

            def prep_S(pr, h0, i, r0, tok):
                zb = zero_bits(tok)
                def A16_(m1, m2, k1, k2):
                    a = wobuf[slot(h0 + k1), (2 * m1 + m2) * DQ + r0:(2 * m1 + m2) * DQ + r0 + RG, k2 * Dh:(k2 + 1) * Dh]
                    return pltpu.bitcast(pltpu.bitcast(a, jnp.uint32) | zb, jnp.bfloat16)
                A16 = memo(A16_)
                A32 = memo(lambda *a: A16(*a).astype(jnp.float32))
                V = memo(lambda m2, k2: lin([(lambda m1=m1, k1=k1: A32(m1, m2, k1, k2), sg) for m1, k1, sg in CA[i]]))
                for j in range(7):
                    if len(CA[i]) == 1 and len(CA[j]) == 1:
                        v = A16(CA[i][0][0], CA[j][0][0], CA[i][0][1], CA[j][0][1])
                    else:
                        v = bf(lin([(lambda m2=m2, k2=k2: V(m2, k2), sg) for m2, k2, sg in CA[j]]))
                    sbuf[pr, 7 * i + j, r0:r0 + RG, :] = v
            def S(pr, i, j, r0, n):
                return pltpu.bitcast(s32[pr, 7 * i + j, r0 // 2:(r0 + n) // 2, :], jnp.bfloat16)

            def put_o(os, k, b, o):
                if ostage:
                    oscr[k, b] = o
                    os[k, b] = lambda r0, r1: oscr[k, b, r0:r1, :]
                else:
                    os[k, b] = lambda r0, r1: o[r0:r1]

            def tile_rows(os, k, r, c, t):
                t0 = t * T
                parts = []
                for g in range(t0 // Sq, (t0 + T - 1) // Sq + 1):
                    a, b = max(t0, g * Sq), min(t0 + T, (g + 1) * Sq)
                    parts.append(os[k, c * CB + g](r * Sq + a - g * Sq, r * Sq + b - g * Sq))
                return jnp.concatenate(parts, axis=0)

            def make_T(os, kbase):
                Bt = lambda k1, k2, n1, n2, t: tile_rows(os, kbase + k1, k2, 2 * n1 + n2, t)
                return memo(lambda i, j, t: bf(lin(diag([(lambda k1=k1, n1=n1, k2=k2, n2=n2: Bt(k1, k2, n1, n2, t), s1 * s2)
                                                         for k1, n1, s1 in CBm[i] for k2, n2, s2 in CBm[j]]))))

            only_a = [i for i in range(7) if all(k1 == 0 for k1, _, _ in CBm[i])]
            rest = [i for i in range(7) if i not in only_a]

            def main_body(h0):
                seq = [c * CB + g for g in range(CB) for c in range(NC)]
                os = {}
                Tm = make_T(os, 0)
                spieces = [(i, r0) for i in only_a + rest for r0 in range(0, DQ, RG)]
                def stream(i, j, t, r0=0, n=DQ):
                    assert all(e[0] != i for e in spieces)
                    y = jax.lax.dot_general(S(0, i, j, r0, n), Tm(i, j, t), NT, preferred_element_type=jnp.float32)
                    old = macc[7 * i + j, t, r0:r0 + n, :]
                    macc[7 * i + j, t, r0:r0 + n, :] = y + jnp.where(h0 > 0, old, 0.0)
                pend = []
                nxt = [0, 0]
                def emit_O(k, p, final=False, cap=None):
                    while nxt[k] < NT3 and NC * (((nxt[k] + 1) * T - 1) // Sq + 1) - 1 <= p:
                        pend.extend((i, j, nxt[k]) for i in (only_a if k == 0 else rest) for j in range(7))
                        nxt[k] += 1
                    nq = 0
                    while len(pend) >= 4 and (cap is None or nq < cap):
                        for _ in range(4):
                            stream(*pend.pop(0))
                        nq += 1
                    if final:
                        X, Y, Z = pend
                        stream(*X, 0, 32); stream(*Y, 0, 64); stream(*X, 32, 112); stream(*Z, 0, 96)
                        stream(*Y, 64, 80); stream(*Z, 96, 48)
                for k in range(2):
                    h = h0 + k
                    s = slot(h)
                    if k == 1:
                        with sc_('mid'):
                            wait_kv(h); wq_cp(h).wait(); wo_cp(h0).wait(); wo_cp(h).wait()
                    ss = {}
                    qpre = {u: ld_q(s, u) for u in seq[:2]}
                    def QK(u):
                        ss[u] = qk(qpre[u] if u in qpre else ld_q(s, u), s, u)
                    def QQ(c):
                        gb = CB // qsplit
                        for j in range(qsplit):
                            toks = Qb(h + LA, c * CB + j * gb, gb, wqbuf.at[s])
                            for r in range(rep):
                                n_ = splan[c] if k == 1 else 0
                                for e in range(n_):
                                    if spieces:
                                        t0 = (e * (gb * Sq // 8) // n_) * 8
                                        prep_S(0, h0, *spieces.pop(0), toks[r][t0:t0 + 8])
                    if k == 0:
                        start_kv(h + LA)
                        wo_cp(h + LA).start(priority=bp); wo_cp(h + 1 + LA).start(priority=bp)
                    else:
                        start_kv(h + LA)
                    QQ(0)
                    wq_cp(h + 1 + LA if k == 0 else h - 1 + LA + 2).start(priority=bp) if False else None
                    if k == 0:
                        wq_cp(h + LA).start(priority=bp); wq_cp(h + 1 + LA).start(priority=bp)
                    QK(seq[0])
                    for i, u in enumerate(seq):
                        if i + 1 < B:
                            QK(seq[i + 1])
                        if i in qpos[k]:
                            QQ(1 + qpos[k].index(i))
                        if k == 1 and i in apos:
                            emit_O(0, B, cap=acap)
                        if k == 1 and i in opos:
                            emit_O(1, i - 1)
                        put_o(os, k, u, pv(ss.pop(u), s, u)[0])
                    QQ(NC - 1)
                emit_O(1, B - 1, final=True)

            def combine_rows(c, t, mq, r0, n, tok=None):
                m1, m2, n1, n2 = mq // 2, mq % 2, c // 2, c % 2
                terms = [(lambda i=i, j=j: macc[7 * i + j, t, r0:r0 + n, :], s1 * s2)
                         for i, s1 in CC[m1][n1] for j, s2 in CC[m2][n2]]
                if tok is not None:
                    zb = zero_bits(tok)
                    zb = jnp.concatenate([zb] * (n // 8), axis=0) if n > 8 else zb
                    th0 = terms[0][0]
                    terms[0] = (lambda: pltpu.bitcast(pltpu.bitcast(th0(), jnp.uint32) | zb, jnp.float32), 1)
                return lin(terms)

            def combine(c, t, pin, toks):
                for mq in range(4):
                    for r0 in range(0, DQ, 8 * pin):
                        base[c * NT3 + t, mq * DQ + r0:mq * DQ + r0 + 8 * pin, :] = combine_rows(c, t, mq, r0, 8 * pin, next(toks))
                return base[c * NT3 + t]

            def tail():
                z = zs[0]
                units = [(hh, c * CB + g) for g in range(CB) for c in range(NC) for hh in range(LA)]
                n = len(units)
                TL = NT3 - 1
                ss, os, raw = {}, {}, {}
                Tm = [make_T(os, 0), make_T(os, 2)]
                spieces = [(pr, H0 + 2 * pr, i, r0) for i in range(7) for r0 in range(0, DQ, RG) for pr in range(2)]
                bpieces = [(c, mq, r0) for c in range(NC) for mq in range(4) for r0 in range(0, DQ, 8 * bpin)]
                outs = []
                fences = {}
                def QK(i):
                    hh, b = units[i]
                    q = q32[slot(H0 + hh), b]
                    for fz in fences.pop(i, []):
                        q = jnp.concatenate([q[0:8] | fz, q[8:]], axis=0)
                    ss[i] = qk(pltpu.bitcast(q, jnp.bfloat16), slot(H0 + hh), b)
                def PV(i):
                    hh, b = units[i]
                    o, raw[i] = pv(ss.pop(i), slot(H0 + hh), b)
                    put_o(os, hh, b, o)
                def stream2(i, j, t, r0=0, n_=DQ):
                    y = lin([(lambda pr=pr: jax.lax.dot_general(S(pr, i, j, r0, n_), Tm[pr](i, j, t), NT,
                                                                preferred_element_type=jnp.float32), 1) for pr in range(2)])
                    macc[7 * i + j, t, r0:r0 + n_, :] += y
                def out_tile(c, t, y, dl=None):
                    tile = c * NT3 + t
                    obuf[tile + z] = bf(y.T)
                    cp = o_cp(tile)
                    cp.start(); outs.append(cp)
                    if dl is not None:
                        obuf[NTL + z, 0:16, 0:T] = jnp.zeros((16, T), obuf.dtype)
                        fences.setdefault(dl, []).append(pltpu.bitcast(obuf[NTL + z, 0:16, 0:T], jnp.uint32))
                def rowtoks(v, step, off=0):
                    return iter([v[r0:r0 + 8] for r0 in range(8 * off, v.shape[0], 8 * step)])
                def Opart(c, hhs):
                    o = jnp.concatenate([bf(tile_rows(os, hh, r, c, TL)) for hh in hhs for r in range(rep)], axis=1)
                    w = jnp.concatenate([wobuf[slot(H0 + hh)] for hh in hhs], axis=1)
                    for fz in fences.pop(('O', c, hhs[0]), []):
                        w0 = pltpu.bitcast(pltpu.bitcast(w[0:16, 0:T], jnp.uint32) | fz, jnp.bfloat16)
                        w = jnp.concatenate([jnp.concatenate([w0, w[0:16, T:]], axis=1), w[16:]], axis=0)
                    return jax.lax.dot_general(w, o, NT, preferred_element_type=jnp.float32)
                def piece(c, dl=None):
                    ya = Opart(c, [0, 1])
                    yb = Opart(c, [2, 3])
                    out_tile(c, TL, (base[c * NT3 + TL] + ya) + yb, dl)
                    return ya, yb
                grp = {t: [(i, j, t) for i in range(7) for j in range(7)] for t in range(TL)}
                gp = {0: g0pos or {33 + e: 4 for e in range(12)}, 1: g1pos or {49 + e: 12 for e in range(4)}}
                ppos = (53, 57, 61)
                QK(0)
                for i in range(n):
                    if i == midbar:
                        with sc_('tmid'):
                            ss[i] = sm(ss[i])
                            wq_cp(Hkv - 1).wait()
                    if i + 1 < n:
                        QK(i + 1)
                    for t in range(TL):
                        for _ in range(gp[t].get(i, 0)):
                            stream2(*grp[t].pop(0))
                        if len(grp[t]) == 1:
                            e = grp[t].pop(0)
                            stream2(*e, 0, 80); stream2(*e, 80, 64)
                    if i in ppos:
                        c = ppos.index(i)
                        ya, yb = piece(c, pdl[c])
                        if c < 2:
                            assert not grp[1]
                            out_tile(2 * c, 1, combine(2 * c, 1, 2, rowtoks(ya, 2)), c1dl[2 * c])
                            out_tile(2 * c + 1, 1, combine(2 * c + 1, 1, 2, rowtoks(yb, 2)), c1dl[2 * c + 1])
                    PV(i)
                    for r0 in range(0, rep * Sq, 8 * tsp):
                        if spieces:
                            prep_S(*spieces.pop(0), raw[i][r0:r0 + 8])
                        for off in boff:
                            if bpieces and i >= bstart:
                                c, mq, rr = bpieces.pop(0)
                                base[c * NT3 + TL, mq * DQ + rr:mq * DQ + rr + 8 * bpin, :] = combine_rows(
                                    c, TL, mq, rr, 8 * bpin, raw[i][r0 + 8 * off:r0 + 8 * off + 8])
                    if c0start <= i < c0start + NC:
                        assert not grp[0]
                        c = i - c0start
                        out_tile(c, 0, combine(c, 0, 3, rowtoks(raw[i], 1)), i + cdl)
                assert not spieces and not bpieces
                piece(NC - 1)
                assert not fences
                with sc_('outw'):
                    for cp in outs:
                        cp.wait()

            x_cp(0).start()
            for hh in range(LA):
                wq0_cp(hh).start()
            for c in range(1, NC):
                x_cp(c).start()
            def bulk():
                for hh in range(0, LA, 2):
                    wq_cp(hh).start(priority=bp0); start_kv(hh, bp0)
                    wo_cp(hh).start(priority=bp0); wo_cp(hh + 1).start(priority=bp0); wq_cp(hh + 1).start(priority=bp0); start_kv(hh + 1, bp0)
            if bulkat == 0:
                bulk()
            zs[0] = 0
            x_cp(0).wait()
            def loop_a(hh, carry):
                with sc_('wa'):
                    wq0_cp(hh).wait()
                with sc_('pa'):
                    Qb(hh, 0, 2, wq0buf.at[hh]); Qb(hh, 2, 2, wq0buf.at[hh])
                return carry
            jax.lax.fori_loop(0, LA, loop_a, 0)
            def loop_b(c, carry):
                with sc_('wb'):
                    x_cp(c).wait()
                with sc_('pb'):
                    for hh in range(LA):
                        Qb(hh, c * CB, CB, wq0buf.at[hh])
                return carry
            jax.lax.fori_loop(1, NC, loop_b, 0)

            def loop_main(i, carry):
                h = 2 * i
                with sc_('wait'):
                    wait_kv(h); wq_cp(h).wait()
                with sc_('body'):
                    main_body(h)
                return carry
            jax.lax.fori_loop(0, H0 // 2, loop_main, 0)
            with sc_('wait'):
                for hh in range(H0, Hkv):
                    wait_kv(hh); wo_cp(hh).wait()
                    if hh < Hkv - 1 or midbar is None:
                        wq_cp(hh).wait()
            with sc_('tail'):
                tail()

        ms = pltpu.HBM
        out = pl.pallas_call(
            kern,
            in_specs=[pl.BlockSpec(memory_space=ms)] * 5,
            out_specs=pl.BlockSpec(memory_space=ms),
            out_shape=jax.ShapeDtypeStruct((M, D), x.dtype),
            scratch_shapes=[
                pltpu.VMEM((M, D), x.dtype),
                pltpu.VMEM((NB, 2, B, Sk, Dh), x.dtype),
                pltpu.VMEM((LA, D, W), x.dtype),
                pltpu.VMEM((NB, D, W), x.dtype),
                pltpu.VMEM((NB, D, W), x.dtype),
                pltpu.VMEM((NB, B, rep * Sq, Dh), x.dtype),
                pltpu.VMEM((2, 49, DQ, Dh), x.dtype),
                pltpu.VMEM((49, NT3, DQ, T), jnp.float32),
                pltpu.VMEM((NTL, D, T), jnp.float32),
                pltpu.VMEM((LA, B, rep * Sq, Dh), jnp.float32),
                pltpu.VMEM((NTL + 1, T, D), x.dtype),
                pltpu.SMEM((1,), jnp.int32),
                pltpu.SemaphoreType.DMA((40 + M // T,)),
            ],
            compiler_params=pltpu.CompilerParams(
                vmem_limit_bytes=vmem * 1024 * 1024, disable_bounds_checks=True, disable_semaphore_checks=True),
        )(x2, k_cache, v_cache, wq, woT)
        return out.reshape(B, Sq, D)
    return f

pallas_standalone__gqa_block_cached__near_ridge_kernel = make()
```

```python
import contextlib

import jax
import jax.numpy as jnp
import jax.experimental.pallas as pl
import jax.experimental.pallas.tpu as pltpu

LOG2E = 1.4426950408889634
NT = (((1,), (1,)), ((), ()))
F32, BF16, U32 = jnp.float32, jnp.bfloat16, jnp.uint32

CA = [[(0, 0, 1), (1, 1, 1)], [(1, 0, 1), (1, 1, 1)], [(0, 0, 1)], [(1, 1, 1)],
      [(0, 0, 1), (0, 1, 1)], [(1, 0, 1), (0, 0, -1)], [(0, 1, 1), (1, 1, -1)]]
CB = [[(0, 0, 1), (1, 1, 1)], [(0, 0, 1)], [(0, 1, 1), (1, 1, -1)], [(1, 0, 1), (0, 0, -1)],
      [(1, 1, 1)], [(0, 0, 1), (0, 1, 1)], [(1, 0, 1), (1, 1, 1)]]
CC = [[[(0, 1), (3, 1), (6, 1), (4, -1)], [(2, 1), (4, 1)]],
      [[(1, 1), (3, 1)], [(0, 1), (2, 1), (5, 1), (1, -1)]]]


def _lin(terms):
    acc = terms[0][0]()
    for th, sg in terms[1:]:
        acc = acc + th() if sg > 0 else acc - th()
    return acc


def _diag(terms):
    return [terms[0], terms[3], terms[1], terms[2]] if len(terms) == 4 else terms


def _memo(fn):
    cache = {}

    def g(*a):
        if a not in cache:
            cache[a] = fn(*a)
        return cache[a]
    return g


def _bf(a):
    return a.astype(BF16)


def _pk(a):
    return pltpu.bitcast(a, U32)


def _zero_bits(tok):
    return jax.lax.shift_right_logical(jax.lax.shift_right_logical(_pk(tok), U32(31)), U32(1))


def make(scopes=False,
         qpos=((7, 8), (2, 12)), opos=(9, 13), apos=(1, 4, 7), acap=4, smp=5, sq=4, spv=5,
         iord=(4, 3, 6, 2, 0, 1, 5), jord=(1, 0, 5, 2, 3, 4, 6), qord=(1, 4, 3, 0, 2, 5, 6),
         g0pos=(34, 6), g1pos=(49, 16), c0start=41, cdl=3, nwin=(28, 4),
         tiord=(4, 6, 5, 2, 0, 3, 1), tjord=(2, 5, 4, 6, 1, 3, 0),
         ppos=(53, 57, 61), pdl=(57, 61, ('O', 3, 2)), c1dl=(58, 59, 62, 63), fsplit=(1, 3, 4)):
    sc_ = jax.named_scope if scopes else (lambda n: contextlib.nullcontext())
    CBT = 4
    LA = 4
    NB = 8
    T = 128
    RG = 16
    LOW = 1

    @jax.jit
    def f(x, k_cache, v_cache, wq, wo):
        B, Sq, D = x.shape
        _, Hkv, Sk, Dh = k_cache.shape
        rep = wq.shape[1] // Dh // Hkv
        assert (B, Sq, D, Hkv, Sk, Dh, rep) == (16, 96, 576, 16, 512, 128, 2)
        scale = (Dh ** -0.5) * LOG2E
        M, W = B * Sq, rep * Dh
        NC, CM = B // CBT, CBT * Sq
        HR = CM // 2
        KC = 3 * T
        KS = (D - KC) // 2
        DQ = D // 4
        NT3 = CM // T
        NTL = M // T
        NQV = rep * Sq // RG
        H0 = Hkv - LA

        def kern(x_hbm, k_hbm, v_hbm, wq_hbm, woT_hbm, o_hbm,
                 x_ref, kvbuf, wq0buf, wqbuf, wobuf, q_ref, xs, sbuf, macc, base, oscr, obuf, zs, sems):
            xsem, kvsem, wq0sem, wqsem, wosem, osem = (
                (lambda i, off=off: sems.at[off + i]) for off in (0, 8, 16, 24, 32, 40))

            def slot(h):
                return h % NB if isinstance(h, int) else jnp.bitwise_and(h, NB - 1)

            def mult(v, m):
                return v if isinstance(v, int) else pl.multiple_of(v, m)

            def x_cp(c):
                rows = pl.ds(mult(c * CM, CM), CM)
                return pltpu.make_async_copy(x_hbm.at[rows], x_ref.at[rows], xsem(c))

            def wq0_cp(h):
                return pltpu.make_async_copy(wq_hbm.at[:, pl.ds(mult(h * W, W), W)], wq0buf.at[h], wq0sem(h))

            def start_kv(h):
                s = slot(h)
                pltpu.make_async_copy(k_hbm.at[:, h], kvbuf.at[s, 0], kvsem(s)).start(priority=LOW)
                pltpu.make_async_copy(v_hbm.at[:, h], kvbuf.at[s, 1], kvsem(s)).start(priority=LOW)

            def wait_kv(h):
                s = slot(h)
                pltpu.make_async_copy(kvbuf.at[s], kvbuf.at[s], kvsem(s)).wait()

            def wq_cp(h):
                hq = min(h + LA, Hkv - 1) if isinstance(h, int) else jnp.minimum(h + LA, Hkv - 1)
                return pltpu.make_async_copy(wq_hbm.at[:, pl.ds(mult(hq * W, W), W)], wqbuf.at[slot(h)], wqsem(slot(h)))

            def wo_cp(h):
                return pltpu.make_async_copy(woT_hbm.at[:, pl.ds(mult(h * W, W), W)], wobuf.at[slot(h)], wosem(slot(h)))

            def put_q(h, b0, r, q):
                q = _bf(q * scale)
                for g in range(q.shape[0] // Sq):
                    q_ref[slot(h), b0 + g, r * Sq // 2:(r + 1) * Sq // 2, :] = _pk(q[g * Sq:(g + 1) * Sq])

            def q_classic(h, b0, gb, w_ref):
                toks = []
                for r in range(rep):
                    q = jnp.dot(x_ref[pl.ds(mult(b0 * Sq, Sq), gb * Sq), :], w_ref[:, r * Dh:(r + 1) * Dh],
                                preferred_element_type=F32)
                    toks.append(q)
                    put_q(h, b0, r, q)
                return toks

            def prep_x(c, r0, tok):
                zb = _zero_bits(tok)

                def blk(m):
                    rows = pl.ds(mult(c * CM + r0 + m * HR, RG), RG)
                    a = pltpu.bitcast(_pk(x_ref[rows, KC:KC + T]) | zb, BF16).astype(F32)
                    v = jnp.concatenate([a, x_ref[rows, KC + T:D].astype(F32)], axis=1)
                    return v[:, :KS], v[:, KS:2 * KS]
                A = [blk(0), blk(1)]
                for i in range(7):
                    v = _lin([(lambda m=m, k=k: A[m][k], sg) for m, k, sg in CA[i]])
                    v = jnp.concatenate([v, jnp.zeros((RG, T - KS), F32)], axis=1)
                    xs[c, i, pl.ds(mult(r0 // 2, RG // 2), RG // 2), :] = _pk(_bf(v))

            def q_strassen(h, c, w_ref):
                Bw = _memo(lambda k, n: w_ref[KC + k * KS:KC + (k + 1) * KS, n * Dh:(n + 1) * Dh])

                @_memo
                def Tq(i):
                    if len(CB[i]) == 1:
                        return Bw(*CB[i][0][:2])
                    return _bf(_lin([(lambda k=k, n=n: Bw(k, n).astype(F32), sg) for k, n, sg in CB[i]]))

                def mp(i, r0, n):
                    a = pltpu.bitcast(xs[c, i, r0 // 2:(r0 + n) // 2, :], BF16)
                    return jnp.dot(a[:, :KS], Tq(i), preferred_element_type=F32)
                Mv = {i: mp(i, 0, HR) for i in qord[:4]}
                X, Y, Z = qord[4:]
                x3, y6a, x9, z9, y6b, z3 = (mp(X, 0, 48), mp(Y, 0, 96), mp(X, 48, 144),
                                            mp(Z, 0, 144), mp(Y, 96, 96), mp(Z, 144, 48))
                Mv[X] = jnp.concatenate([x3, x9], axis=0)
                Mv[Y] = jnp.concatenate([y6a, y6b], axis=0)
                Mv[Z] = jnp.concatenate([z9, z3], axis=0)
                toks = [Mv[qord[0]], x9]
                for m in range(2):
                    for r in range(rep):
                        q = jnp.dot(x_ref[pl.ds(mult(c * CM + m * HR, HR), HR), :KC], w_ref[:KC, r * Dh:(r + 1) * Dh],
                                    preferred_element_type=F32)
                        q = q + _lin([(lambda i=i: Mv[i], sg) for i, sg in CC[m][r]])
                        toks.append(q)
                        put_q(h, c * CBT + m * (CBT // 2), r, q)
                return toks

            def qk(q32, s, b):
                return jax.lax.dot_general(pltpu.bitcast(q32, BF16), kvbuf[s, 0, b], NT, preferred_element_type=F32)

            def pv(sc, s, b):
                m = jnp.max(sc, axis=-1, keepdims=True)
                p = jnp.exp2(sc - m)
                pt = [p[:, t * T:(t + 1) * T] for t in range(Sk // T)]
                ps = pt[0]
                for t in range(1, Sk // T):
                    ps = ps + pt[t]
                pt[-1] = jnp.minimum(pt[-1], ps)
                p = _bf(jnp.concatenate(pt, axis=1))
                l = jnp.sum(ps, axis=-1, keepdims=True)
                o = jnp.dot(p, kvbuf[s, 1, b], preferred_element_type=F32)
                r = pl.reciprocal(l, approx=True)
                r = r * (2.0 - l * r)
                return o * r, o, jnp.broadcast_to(l, o.shape)

            def put_o(done, k, b, o):
                c, g = divmod(b, CBT)
                for r in range(rep):
                    oscr[k, r, c, g * Sq:(g + 1) * Sq, :] = o[r * Sq:(r + 1) * Sq]
                done.add((k, b))

            def o_tile(done, k, r, c, t):
                assert all((k, c * CBT + g) in done for g in range(t * T // Sq, (t * T + T - 1) // Sq + 1))
                return oscr[k, r, c, t * T:(t + 1) * T, :]

            def prep_s(pr, h0, i, r0, tok):
                zb = jnp.concatenate([_zero_bits(tok)] * rep, axis=1)

                @_memo
                def Aw(m1, m2, k1):
                    a = wobuf[slot(h0 + k1), (2 * m1 + m2) * DQ + r0:(2 * m1 + m2) * DQ + r0 + RG, :]
                    return pltpu.bitcast(_pk(a) | zb, BF16)
                A16 = lambda m1, m2, k1, k2: Aw(m1, m2, k1)[:, k2 * Dh:(k2 + 1) * Dh]
                A32 = _memo(lambda *a: A16(*a).astype(F32))
                V = _memo(lambda m2, k2: _lin([(lambda m1=m1, k1=k1: A32(m1, m2, k1, k2), sg) for m1, k1, sg in CA[i]]))
                vs = []
                for j in range(7):
                    if len(CA[i]) == 1 and len(CA[j]) == 1:
                        v = A16(CA[i][0][0], CA[j][0][0], CA[i][0][1], CA[j][0][1])
                    else:
                        v = _bf(_lin([(lambda m2=m2, k2=k2: V(m2, k2), sg) for m2, k2, sg in CA[j]]))
                    vs.append(_pk(v))
                sbuf[pr, 7 * i:7 * i + 7, r0 // 2:(r0 + RG) // 2, :] = jnp.stack(vs)

            def s_op(pr, i, j, r0, n):
                return pltpu.bitcast(sbuf[pr, 7 * i + j, r0 // 2:(r0 + n) // 2, :], BF16)

            def make_t(done, kbase):
                return _memo(lambda i, j, t: _bf(_lin(_diag(
                    [(lambda k1=k1, n1=n1, k2=k2, n2=n2: o_tile(done, kbase + k1, k2, 2 * n1 + n2, t), s1 * s2)
                     for k1, n1, s1 in CB[i] for k2, n2, s2 in CB[j]]))))

            def combine_rows(c, t, mq, r0, tok=None):
                blk = macc[t, r0 // RG]
                terms = [(lambda i=i, j=j: blk[7 * i + j], s1 * s2)
                         for i, s1 in CC[mq // 2][c // 2] for j, s2 in CC[mq % 2][c % 2]]
                if tok is not None:
                    zb = jnp.concatenate([_zero_bits(tok)] * 2, axis=0)
                    th0 = terms[0][0]
                    terms[0] = (lambda: pltpu.bitcast(_pk(th0()) | zb, F32), 1)
                v = _lin(terms)
                base[c * NT3 + t, mq * DQ + r0:mq * DQ + r0 + RG, :] = v
                return v

            first_only = [i for i in range(7) if all(k1 == 0 for k1, _, _ in CB[i])]

            def main_body(h0):
                seq = [c * CBT + g for g in range(CBT) for c in range(NC)]
                done = set()
                Tm = make_t(done, 0)
                spieces = [(i, r0) for i in sorted(iord, key=lambda i: i not in first_only) for r0 in range(0, DQ, RG)]
                pend, nxt = [], [0, 0]

                def pin_s(tk, n):
                    for e in range(n):
                        if spieces:
                            t0 = (e * (tk.shape[0] // 8) // n) * 8
                            prep_s(0, h0, *spieces.pop(0), tk[t0:t0 + 8])

                def stream(i, j, t, r0=0, n=DQ):
                    assert all(e[0] != i for e in spieces)
                    y = jax.lax.dot_general(s_op(0, i, j, r0, n), Tm(i, j, t), NT, preferred_element_type=F32)
                    old = macc[t, r0 // RG:(r0 + n) // RG, 7 * i + j]
                    macc[t, r0 // RG:(r0 + n) // RG, 7 * i + j] = y.reshape(old.shape) + jnp.where(h0 > 0, old, 0.0)

                def emit_o(k, p, cap=None):
                    while nxt[k] < NT3 and NC * (((nxt[k] + 1) * T - 1) // Sq + 1) - 1 <= p:
                        pend.extend((i, j, nxt[k]) for i in iord if (i in first_only) == (k == 0) for j in jord)
                        nxt[k] += 1
                    nq = 0
                    while len(pend) >= 4 and (cap is None or nq < cap):
                        for _ in range(4):
                            stream(*pend.pop(0))
                        nq += 1

                for k in range(2):
                    h = h0 + k
                    s = slot(h)
                    if k == 1:
                        with sc_('mid'):
                            wait_kv(h); wq_cp(h).wait(); wo_cp(h0).wait(); wo_cp(h).wait()
                    ss = {}
                    qpre = {u: q_ref[s, u] for u in seq[:2]}

                    def QK(u):
                        ss[u] = qk(qpre[u] if u in qpre else q_ref[s, u], s, u)

                    def QQ(c):
                        toks = q_strassen(h + LA, c, wqbuf.at[s])
                        if k == 1 and c == 0:
                            for a, tk in enumerate(toks):
                                pin_s(tk, smp if a < 2 else sq)
                    start_kv(h + LA)
                    if k == 0:
                        wo_cp(h + LA).start(priority=LOW); wo_cp(h + 1 + LA).start(priority=LOW)
                    QQ(0)
                    if k == 0:
                        wq_cp(h + LA).start(priority=LOW); wq_cp(h + 1 + LA).start(priority=LOW)
                    QK(seq[0])
                    for i, u in enumerate(seq):
                        if i + 1 < B:
                            QK(seq[i + 1])
                        if i in qpos[k]:
                            QQ(1 + qpos[k].index(i))
                        if k == 1 and i in apos:
                            emit_o(0, B, cap=acap)
                        if k == 1 and i in opos:
                            emit_o(1, i - 1)
                        o, raw, _ = pv(ss.pop(u), s, u)
                        put_o(done, k, u, o)
                        if k == 1:
                            pin_s(raw, spv)
                    QQ(NC - 1)
                emit_o(1, B - 1)
                X, Y, Z = pend
                stream(*X, 0, 32); stream(*Y, 0, 64); stream(*X, 32, 112); stream(*Z, 0, 96)
                stream(*Y, 64, 80); stream(*Z, 96, 48)

            def tail():
                z = zs[0]
                units = [(hh, c * CBT + g) for g in range(CBT) for c in range(NC) for hh in range(LA)]
                n = len(units)
                TL = NT3 - 1
                ss, raw, done = {}, {}, set()
                Tm = [make_t(done, 0), make_t(done, 2)]
                spieces = [(pr, H0 + 2 * pr, i, r0) for i in range(7) for r0 in range(0, DQ, RG) for pr in range(2)]
                bpieces = [(c, TL, mq, r0) for c in range(NC) for mq in range(4) for r0 in range(0, DQ, RG)]
                grp = {t: [(i, j, t) for i in tiord for j in tjord] for t in range(TL)}
                gp = [{st + e: per for e in range(48 // per)} for st, per in (g0pos, g1pos)]
                outs, fences, dls = [], {}, {}

                def deadline(i, j, v):
                    dls.setdefault(i, {}).setdefault(j, []).append(v)

                def fenced16(a, key):
                    for fz in fences.pop(key, []):
                        a0 = pltpu.bitcast(_pk(a[0:RG, 0:T]) | fz, BF16)
                        a = jnp.concatenate([jnp.concatenate([a0, a[0:RG, T:]], axis=1), a[RG:]], axis=0)
                    return a

                def QK(i):
                    hh, b = units[i]
                    q = q_ref[slot(H0 + hh), b]
                    for fz in fences.pop(i, []):
                        q = jnp.concatenate([q[0:8] | fz, q[8:]], axis=0)
                    deps = dls.pop(i, None)
                    if deps:
                        parts = []
                        for j in range(NQV):
                            v = q[8 * j:8 * j + 8]
                            us = [_pk(d[r:r + 8]) for d in deps.get(j, []) for r in range(0, d.shape[0], 8)]
                            if us:
                                u = us[0]
                                for w in us[1:]:
                                    u = u | w
                                v = v | _zero_bits(u)
                            parts.append(v)
                        q = jnp.concatenate(parts, axis=0)
                    ss[i] = qk(q, slot(H0 + hh), b)

                def PV(i):
                    hh, b = units[i]
                    o, raw[i], lb = pv(ss.pop(i), slot(H0 + hh), b)
                    put_o(done, hh, b, o)
                    if i < nwin[0]:
                        for j in range(NQV):
                            deadline(i + nwin[1], j, lb[RG * j:RG * j + RG])

                def stream2(i, j, t, r0=0, nr=DQ):
                    y = _lin([(lambda pr=pr: jax.lax.dot_general(s_op(pr, i, j, r0, nr), Tm[pr](i, j, t), NT,
                                                                 preferred_element_type=F32), 1) for pr in range(2)])
                    macc[t, r0 // RG:(r0 + nr) // RG, 7 * i + j] += y.reshape(nr // RG, RG, T)

                def out_tile(c, t, y, dl, bslots=None):
                    tile = c * NT3 + t
                    if bslots is None:
                        obuf[tile + z] = _bf(y.T)
                    else:
                        for d0 in range(0, D, T):
                            d1 = min(D, d0 + T)
                            v = _bf(y[d0:d1].T)
                            obuf[tile + z, :, d0:d1] = v
                            if d1 - d0 == T:
                                deadline(*next(bslots), _pk(v))
                    cp = pltpu.make_async_copy(obuf.at[tile], o_hbm.at[pl.ds(tile * T, T)], osem(tile))
                    cp.start()
                    outs.append(cp)
                    obuf[NTL + z, 0:RG, 0:T] = jnp.zeros((RG, T), obuf.dtype)
                    fences.setdefault(dl, []).append(_pk(obuf[NTL + z, 0:RG, 0:T]))

                def combine(c, t, toks=None, slots=None):
                    for mq in range(4):
                        for r0 in range(0, DQ, RG):
                            v = combine_rows(c, t, mq, r0, next(toks) if toks is not None else None)
                            if slots is not None:
                                deadline(*next(slots), v)
                    return base[c * NT3 + t]

                def o_cols(c, hhs):
                    return jnp.concatenate([_bf(o_tile(done, hh, r, c, TL)) for hh in hhs for r in range(rep)], axis=1)

                def o_classic(c, hhs):
                    o = o_cols(c, hhs)
                    w = jnp.concatenate([wobuf[slot(H0 + hh)] for hh in hhs], axis=1)
                    return jax.lax.dot_general(fenced16(w, ('O', c, hhs[0])), o, NT, preferred_element_type=F32)

                QK(0)
                for i in range(n):
                    if i + 1 < n:
                        QK(i + 1)
                    for t in range(TL):
                        for _ in range(gp[t].get(i, 0)):
                            stream2(*grp[t].pop(0))
                        if len(grp[t]) == 1:
                            e = grp[t].pop(0)
                            stream2(*e, 0, 80); stream2(*e, 80, 64)
                    if i in ppos:
                        c = ppos.index(i)
                        ya, yb = o_classic(c, [0, 1]), o_classic(c, [2, 3])
                        out_tile(c, TL, (base[c * NT3 + TL] + ya) + yb, pdl[c])
                        if c < 2:
                            assert not grp[1]
                            for cc, y in ((2 * c, ya), (2 * c + 1, yb)):
                                toks = iter([y[r0:r0 + 8] for r0 in range(0, D, RG)])
                                out_tile(cc, 1, combine(cc, 1, toks=toks), c1dl[cc])
                    PV(i)
                    for r0 in range(0, rep * Sq, 48):
                        if spieces:
                            prep_s(*spieces.pop(0), raw[i][r0:r0 + 8])
                        for off in (16, 32):
                            if bpieces:
                                combine_rows(*bpieces.pop(0), raw[i][r0 + off:r0 + off + 8])
                    if i == c0start:
                        assert not grp[0]
                        slots = iter([(ii, j) for ii in range(i + 2, n) for j in range(NQV)])
                        for c in range(NC):
                            e0 = i + 2 + ((c + 1) * (D // RG) - 1) // NQV
                            bs = iter([(e0 + 1 + a // 2, 3 + 6 * (a % 2)) for a in range(4)])
                            out_tile(c, 0, combine(c, 0, slots=slots), e0 + cdl, bs)
                assert not spieces and not bpieces
                c = NC - 1
                tile = c * NT3 + TL
                pre = (base[tile] + o_classic(c, [0, 1])).T
                o = fenced16(o_cols(c, [2, 3]), ('O', c, 2))
                lo = 0
                for e, d0 in enumerate(range(0, D, T)):
                    d1 = min(D, d0 + T)
                    w = jnp.concatenate([wobuf[slot(H0 + hh), d0:d1, :] for hh in (2, 3)], axis=1)
                    yb = jax.lax.dot_general(o, w, NT, preferred_element_type=F32)
                    obuf[tile + z, :, d0:d1] = _bf(pre[:, d0:d1] + yb)
                    if e in fsplit:
                        cols = pl.ds(lo, d1 - lo)
                        cp = pltpu.make_async_copy(obuf.at[tile, :, cols], o_hbm.at[pl.ds(tile * T, T), cols],
                                                   osem(tile + fsplit.index(e)))
                        cp.start()
                        outs.append(cp)
                        lo = d1
                assert not fences and not dls and lo == D
                with sc_('outw'):
                    for cp in outs:
                        cp.wait()

            x_cp(0).start()
            for hh in range(LA):
                wq0_cp(hh).start()
            for c in range(1, NC):
                x_cp(c).start()
            for hh in range(0, LA, 2):
                wq_cp(hh).start(priority=LOW); start_kv(hh)
                wo_cp(hh).start(priority=LOW); wo_cp(hh + 1).start(priority=LOW)
                wq_cp(hh + 1).start(priority=LOW); start_kv(hh + 1)
            zs[0] = 0
            x_cp(0).wait()

            def loop_a(hh, carry):
                with sc_('wa'):
                    wq0_cp(hh).wait()
                with sc_('pa'):
                    q_classic(hh, 0, 2, wq0buf.at[hh]); q_classic(hh, 2, 2, wq0buf.at[hh])
                return carry
            jax.lax.fori_loop(0, LA, loop_a, 0)

            def loop_b(c, carry):
                with sc_('wb'):
                    x_cp(c).wait()
                with sc_('pb'):
                    toks = q_classic(0, c * CBT, CBT, wq0buf.at[0]) + q_classic(1, c * CBT, CBT, wq0buf.at[1])
                    for e, r0 in enumerate(range(0, HR, RG)):
                        t0 = (e % 4) * (CM // 4)
                        prep_x(c, r0, toks[e // 4][t0:t0 + 8])
                    for hh in range(2, LA):
                        toks += q_strassen(hh, c, wq0buf.at[hh])[2:]
                    r3 = HR // (NC - 1)
                    for e, r0 in enumerate(range(0, r3, RG)):
                        prep_x(0, (c - 1) * r3 + r0, toks[-1 - e][0:8])
                return carry
            jax.lax.fori_loop(1, NC, loop_b, 0)

            def loop_main(i, carry):
                with sc_('wait'):
                    wait_kv(2 * i); wq_cp(2 * i).wait()
                with sc_('body'):
                    main_body(2 * i)
                return carry
            jax.lax.fori_loop(0, H0 // 2, loop_main, 0)
            with sc_('wait'):
                for hh in range(H0, Hkv):
                    wait_kv(hh); wo_cp(hh).wait(); wq_cp(hh).wait()
            with sc_('tail'):
                tail()

        hbm = pl.BlockSpec(memory_space=pltpu.HBM)
        out = pl.pallas_call(
            kern,
            in_specs=[hbm] * 5,
            out_specs=hbm,
            out_shape=jax.ShapeDtypeStruct((M, D), x.dtype),
            scratch_shapes=[
                pltpu.VMEM((M, D), BF16),
                pltpu.VMEM((NB, 2, B, Sk, Dh), BF16),
                pltpu.VMEM((LA, D, W), BF16),
                pltpu.VMEM((NB, D, W), BF16),
                pltpu.VMEM((NB, D, W), BF16),
                pltpu.VMEM((NB, B, rep * Sq // 2, Dh), U32),
                pltpu.VMEM((NC, 7, HR // 2, T), U32),
                pltpu.VMEM((2, 49, DQ // 2, Dh), U32),
                pltpu.VMEM((NT3, DQ // RG, 49, RG, T), F32),
                pltpu.VMEM((NTL, D, T), F32),
                pltpu.VMEM((LA, rep, NC, CM, Dh), F32),
                pltpu.VMEM((NTL + 1, T, D), BF16),
                pltpu.SMEM((1,), jnp.int32),
                pltpu.SemaphoreType.DMA((40 + NTL + len(fsplit),)),
            ],
            compiler_params=pltpu.CompilerParams(
                vmem_limit_bytes=100 * 1024 * 1024,
                disable_bounds_checks=True, disable_semaphore_checks=True),
        )(x.reshape(M, D), k_cache, v_cache, wq, wo.T)
        return out.reshape(B, Sq, D)
    return f


pallas_standalone__gqa_block_cached__near_ridge_kernel = make()
```

```python
import contextlib

import jax
import jax.numpy as jnp
import jax.experimental.pallas as pl
import jax.experimental.pallas.tpu as pltpu

LOG2E = 1.4426950408889634
NT = (((1,), (1,)), ((), ()))
F32, BF16, U32 = jnp.float32, jnp.bfloat16, jnp.uint32

CA = [[(0, 0, 1), (1, 1, 1)], [(1, 0, 1), (1, 1, 1)], [(0, 0, 1)], [(1, 1, 1)],
      [(0, 0, 1), (0, 1, 1)], [(1, 0, 1), (0, 0, -1)], [(0, 1, 1), (1, 1, -1)]]
CB = [[(0, 0, 1), (1, 1, 1)], [(0, 0, 1)], [(0, 1, 1), (1, 1, -1)], [(1, 0, 1), (0, 0, -1)],
      [(1, 1, 1)], [(0, 0, 1), (0, 1, 1)], [(1, 0, 1), (1, 1, 1)]]
CC = [[[(0, 1), (3, 1), (6, 1), (4, -1)], [(2, 1), (4, 1)]],
      [[(1, 1), (3, 1)], [(0, 1), (2, 1), (5, 1), (1, -1)]]]


def _lin(terms):
    acc = terms[0][0]()
    for th, sg in terms[1:]:
        acc = acc + th() if sg > 0 else acc - th()
    return acc


def _diag(terms):
    return [terms[0], terms[3], terms[1], terms[2]] if len(terms) == 4 else terms


def _memo(fn):
    cache = {}

    def g(*a):
        if a not in cache:
            cache[a] = fn(*a)
        return cache[a]
    return g


def _bf(a):
    return a.astype(BF16)


def _pk(a):
    return pltpu.bitcast(a, U32)


def _zero_bits(tok):
    return jax.lax.shift_right_logical(jax.lax.shift_right_logical(_pk(tok), U32(31)), U32(1))


def make(scopes=False,
         qpos=((8, 10), (5, 12)), opos=(9, 13), apos=(1, 4, 7), acap=4, smp=5, sq=4, spv=5,
         iord=(4, 3, 2, 6, 0, 1, 5), jord=(1, 0, 5, 6, 4, 2, 3), qord=(1, 6, 3, 0, 2, 5, 4),
         g0pos=(34, 6), g1pos=(50, 16), c0start=41, cdl=3, nwin=(26, 5),
         tiord=(4, 3, 0, 2, 5, 1, 6), tjord=(2, 5, 0, 6, 1, 3, 4),
         ppos=(53, 57, 62), pdl=(57, 61, ('O', 3, 2)), c1dl=(58, 59, 62, 63), fsplit=(1, 3, 4)):
    sc_ = jax.named_scope if scopes else (lambda n: contextlib.nullcontext())
    CBT = 4
    LA = 4
    NB = 8
    T = 128
    RG = 16
    LOW = 1

    @jax.jit
    def f(x, k_cache, v_cache, wq, wo):
        B, Sq, D = x.shape
        _, Hkv, Sk, Dh = k_cache.shape
        rep = wq.shape[1] // Dh // Hkv
        assert (B, Sq, D, Hkv, Sk, Dh, rep) == (16, 96, 576, 16, 512, 128, 2)
        scale = (Dh ** -0.5) * LOG2E
        M, W = B * Sq, rep * Dh
        NC, CM = B // CBT, CBT * Sq
        HR = CM // 2
        KC = 3 * T
        KS = (D - KC) // 2
        DQ = D // 4
        NT3 = CM // T
        NTL = M // T
        NQV = rep * Sq // RG
        H0 = Hkv - LA

        def kern(x_hbm, k_hbm, v_hbm, wq_hbm, woT_hbm, o_hbm,
                 x_ref, kvbuf, wq0buf, wqbuf, wobuf, q_ref, xs, sbuf, macc, base, oscr, obuf, zs, sems):
            xsem, kvsem, wq0sem, wqsem, wosem, osem = (
                (lambda i, off=off: sems.at[off + i]) for off in (0, 8, 16, 24, 32, 40))

            def slot(h):
                return h % NB if isinstance(h, int) else jnp.bitwise_and(h, NB - 1)

            def mult(v, m):
                return v if isinstance(v, int) else pl.multiple_of(v, m)

            def x_cp(c):
                rows = pl.ds(mult(c * CM, CM), CM)
                return pltpu.make_async_copy(x_hbm.at[rows], x_ref.at[rows], xsem(c))

            def wq0_cp(h):
                return pltpu.make_async_copy(wq_hbm.at[:, pl.ds(mult(h * W, W), W)], wq0buf.at[h], wq0sem(h))

            def start_kv(h):
                s = slot(h)
                pltpu.make_async_copy(k_hbm.at[:, h], kvbuf.at[s, 0], kvsem(s)).start(priority=LOW)
                pltpu.make_async_copy(v_hbm.at[:, h], kvbuf.at[s, 1], kvsem(s)).start(priority=LOW)

            def wait_kv(h):
                s = slot(h)
                pltpu.make_async_copy(kvbuf.at[s], kvbuf.at[s], kvsem(s)).wait()

            def wq_cp(h):
                hq = min(h + LA, Hkv - 1) if isinstance(h, int) else jnp.minimum(h + LA, Hkv - 1)
                return pltpu.make_async_copy(wq_hbm.at[:, pl.ds(mult(hq * W, W), W)], wqbuf.at[slot(h)], wqsem(slot(h)))

            def wo_cp(h):
                return pltpu.make_async_copy(woT_hbm.at[:, pl.ds(mult(h * W, W), W)], wobuf.at[slot(h)], wosem(slot(h)))

            def put_q(h, b0, r, q):
                q = _bf(q * scale)
                for g in range(q.shape[0] // Sq):
                    q_ref[slot(h), b0 + g, r * Sq // 2:(r + 1) * Sq // 2, :] = _pk(q[g * Sq:(g + 1) * Sq])

            def q_classic(h, b0, gb, w_ref):
                toks = []
                for r in range(rep):
                    q = jnp.dot(x_ref[pl.ds(mult(b0 * Sq, Sq), gb * Sq), :], w_ref[:, r * Dh:(r + 1) * Dh],
                                preferred_element_type=F32)
                    toks.append(q)
                    put_q(h, b0, r, q)
                return toks

            def prep_x(c, r0, tok):
                zb = _zero_bits(tok)

                def blk(m):
                    rows = pl.ds(mult(c * CM + r0 + m * HR, RG), RG)
                    a = pltpu.bitcast(_pk(x_ref[rows, KC:KC + T]) | zb, BF16).astype(F32)
                    v = jnp.concatenate([a, x_ref[rows, KC + T:D].astype(F32)], axis=1)
                    return v[:, :KS], v[:, KS:2 * KS]
                A = [blk(0), blk(1)]
                for i in range(7):
                    v = _lin([(lambda m=m, k=k: A[m][k], sg) for m, k, sg in CA[i]])
                    v = jnp.concatenate([v, jnp.zeros((RG, T - KS), F32)], axis=1)
                    xs[c, i, pl.ds(mult(r0 // 2, RG // 2), RG // 2), :] = _pk(_bf(v))

            def q_strassen(h, c, w_ref):
                Bw = _memo(lambda k, n: w_ref[KC + k * KS:KC + (k + 1) * KS, n * Dh:(n + 1) * Dh])

                @_memo
                def Tq(i):
                    if len(CB[i]) == 1:
                        return Bw(*CB[i][0][:2])
                    return _bf(_lin([(lambda k=k, n=n: Bw(k, n).astype(F32), sg) for k, n, sg in CB[i]]))

                def mp(i, r0, n):
                    a = pltpu.bitcast(xs[c, i, r0 // 2:(r0 + n) // 2, :], BF16)
                    return jnp.dot(a[:, :KS], Tq(i), preferred_element_type=F32)
                Mv = {i: mp(i, 0, HR) for i in qord[:4]}
                X, Y, Z = qord[4:]
                x3, y6a, x9, z9, y6b, z3 = (mp(X, 0, 48), mp(Y, 0, 96), mp(X, 48, 144),
                                            mp(Z, 0, 144), mp(Y, 96, 96), mp(Z, 144, 48))
                Mv[X] = jnp.concatenate([x3, x9], axis=0)
                Mv[Y] = jnp.concatenate([y6a, y6b], axis=0)
                Mv[Z] = jnp.concatenate([z9, z3], axis=0)
                toks = [Mv[qord[0]], x9]
                for m in range(2):
                    for r in range(rep):
                        q = jnp.dot(x_ref[pl.ds(mult(c * CM + m * HR, HR), HR), :KC], w_ref[:KC, r * Dh:(r + 1) * Dh],
                                    preferred_element_type=F32)
                        q = q + _lin([(lambda i=i: Mv[i], sg) for i, sg in CC[m][r]])
                        toks.append(q)
                        put_q(h, c * CBT + m * (CBT // 2), r, q)
                return toks

            def qk(q32, s, b):
                return jax.lax.dot_general(pltpu.bitcast(q32, BF16), kvbuf[s, 0, b], NT, preferred_element_type=F32)

            def pv(sc, s, b):
                m = jnp.max(sc, axis=-1, keepdims=True)
                p = jnp.exp2(sc - m)
                pt = [p[:, t * T:(t + 1) * T] for t in range(Sk // T)]
                ps = pt[0]
                for t in range(1, Sk // T):
                    ps = ps + pt[t]
                pt[-1] = jnp.minimum(pt[-1], ps)
                p = _bf(jnp.concatenate(pt, axis=1))
                l = jnp.sum(ps, axis=-1, keepdims=True)
                o = jnp.dot(p, kvbuf[s, 1, b], preferred_element_type=F32)
                r = pl.reciprocal(l, approx=True)
                r = r * (2.0 - l * r)
                return o * r, o, jnp.broadcast_to(l, o.shape)

            def put_o(done, k, b, o):
                c, g = divmod(b, CBT)
                for r in range(rep):
                    oscr[k, r, c, g * Sq:(g + 1) * Sq, :] = o[r * Sq:(r + 1) * Sq]
                done.add((k, b))

            def o_tile(done, k, r, c, t):
                assert all((k, c * CBT + g) in done for g in range(t * T // Sq, (t * T + T - 1) // Sq + 1))
                return oscr[k, r, c, t * T:(t + 1) * T, :]

            def prep_s(pr, h0, i, r0, tok):
                zb = jnp.concatenate([_zero_bits(tok)] * rep, axis=1)

                @_memo
                def Aw(m1, m2, k1):
                    a = wobuf[slot(h0 + k1), (2 * m1 + m2) * DQ + r0:(2 * m1 + m2) * DQ + r0 + RG, :]
                    return pltpu.bitcast(_pk(a) | zb, BF16)
                A16 = lambda m1, m2, k1, k2: Aw(m1, m2, k1)[:, k2 * Dh:(k2 + 1) * Dh]
                A32 = _memo(lambda *a: A16(*a).astype(F32))
                V = _memo(lambda m2, k2: _lin([(lambda m1=m1, k1=k1: A32(m1, m2, k1, k2), sg) for m1, k1, sg in CA[i]]))
                vs = []
                for j in range(7):
                    if len(CA[i]) == 1 and len(CA[j]) == 1:
                        v = A16(CA[i][0][0], CA[j][0][0], CA[i][0][1], CA[j][0][1])
                    else:
                        v = _bf(_lin([(lambda m2=m2, k2=k2: V(m2, k2), sg) for m2, k2, sg in CA[j]]))
                    vs.append(_pk(v))
                sbuf[pr, 7 * i:7 * i + 7, r0 // 2:(r0 + RG) // 2, :] = jnp.stack(vs)

            def s_op(pr, i, j, r0, n):
                return pltpu.bitcast(sbuf[pr, 7 * i + j, r0 // 2:(r0 + n) // 2, :], BF16)

            def make_t(done, kbase):
                return _memo(lambda i, j, t: _bf(_lin(_diag(
                    [(lambda k1=k1, n1=n1, k2=k2, n2=n2: o_tile(done, kbase + k1, k2, 2 * n1 + n2, t), s1 * s2)
                     for k1, n1, s1 in CB[i] for k2, n2, s2 in CB[j]]))))

            def combine_rows(c, t, mq, r0, tok=None):
                blk = macc[t, r0 // RG]
                terms = [(lambda i=i, j=j: blk[7 * i + j], s1 * s2)
                         for i, s1 in CC[mq // 2][c // 2] for j, s2 in CC[mq % 2][c % 2]]
                if tok is not None:
                    zb = jnp.concatenate([_zero_bits(tok)] * 2, axis=0)
                    th0 = terms[0][0]
                    terms[0] = (lambda: pltpu.bitcast(_pk(th0()) | zb, F32), 1)
                v = _lin(terms)
                base[c * NT3 + t, mq * DQ + r0:mq * DQ + r0 + RG, :] = v
                return v

            first_only = [i for i in range(7) if all(k1 == 0 for k1, _, _ in CB[i])]

            def main_body(h0):
                seq = [c * CBT + g for g in range(CBT) for c in range(NC)]
                done = set()
                Tm = make_t(done, 0)
                spieces = [(i, r0) for i in sorted(iord, key=lambda i: i not in first_only) for r0 in range(0, DQ, RG)]
                pend, nxt = [], [0, 0]

                def pin_s(tk, n):
                    for e in range(n):
                        if spieces:
                            t0 = (e * (tk.shape[0] // 8) // n) * 8
                            prep_s(0, h0, *spieces.pop(0), tk[t0:t0 + 8])

                def stream(i, j, t, r0=0, n=DQ):
                    assert all(e[0] != i for e in spieces)
                    y = jax.lax.dot_general(s_op(0, i, j, r0, n), Tm(i, j, t), NT, preferred_element_type=F32)
                    old = macc[t, r0 // RG:(r0 + n) // RG, 7 * i + j]
                    macc[t, r0 // RG:(r0 + n) // RG, 7 * i + j] = y.reshape(old.shape) + jnp.where(h0 > 0, old, 0.0)

                def emit_o(k, p, cap=None):
                    while nxt[k] < NT3 and NC * (((nxt[k] + 1) * T - 1) // Sq + 1) - 1 <= p:
                        pend.extend((i, j, nxt[k]) for i in iord if (i in first_only) == (k == 0) for j in jord)
                        nxt[k] += 1
                    nq = 0
                    while len(pend) >= 4 and (cap is None or nq < cap):
                        for _ in range(4):
                            stream(*pend.pop(0))
                        nq += 1

                for k in range(2):
                    h = h0 + k
                    s = slot(h)
                    if k == 1:
                        with sc_('mid'):
                            wait_kv(h); wq_cp(h).wait(); wo_cp(h0).wait(); wo_cp(h).wait()
                    ss = {}
                    qpre = {u: q_ref[s, u] for u in seq[:2]}

                    def QK(u):
                        ss[u] = qk(qpre[u] if u in qpre else q_ref[s, u], s, u)

                    def QQ(c):
                        toks = q_strassen(h + LA, c, wqbuf.at[s])
                        if k == 1 and c == 0:
                            for a, tk in enumerate(toks):
                                pin_s(tk, smp if a < 2 else sq)
                    start_kv(h + LA)
                    if k == 0:
                        wo_cp(h + LA).start(priority=LOW); wo_cp(h + 1 + LA).start(priority=LOW)
                    QQ(0)
                    if k == 0:
                        wq_cp(h + LA).start(priority=LOW); wq_cp(h + 1 + LA).start(priority=LOW)
                    QK(seq[0])
                    for i, u in enumerate(seq):
                        if i + 1 < B:
                            QK(seq[i + 1])
                        if i in qpos[k]:
                            QQ(1 + qpos[k].index(i))
                        if k == 1 and i in apos:
                            emit_o(0, B, cap=acap)
                        if k == 1 and i in opos:
                            emit_o(1, i - 1)
                        o, raw, _ = pv(ss.pop(u), s, u)
                        put_o(done, k, u, o)
                        if k == 1:
                            pin_s(raw, spv)
                    QQ(NC - 1)
                emit_o(1, B - 1)
                X, Y, Z = pend
                stream(*X, 0, 32); stream(*Y, 0, 64); stream(*X, 32, 112); stream(*Z, 0, 96)
                stream(*Y, 64, 80); stream(*Z, 96, 48)

            def tail():
                z = zs[0]

                def dyn(i):
                    return jnp.minimum(jnp.maximum(i + z, i), i)
                units = [(hh, c * CBT + g) for g in range(CBT) for c in range(NC) for hh in range(LA)]
                n = len(units)
                TL = NT3 - 1
                ss, raw, done = {}, {}, set()
                Tm = [make_t(done, 0), make_t(done, 2)]
                spieces = [(pr, H0 + 2 * pr, i, r0) for i in range(7) for r0 in range(0, DQ, RG) for pr in range(2)]
                bpieces = [(c, TL, mq, r0) for c in range(NC) for mq in range(4) for r0 in range(0, DQ, RG)]
                grp = {t: [(i, j, t) for i in tiord for j in tjord] for t in range(TL)}
                gp = [{st + e: per for e in range(48 // per)} for st, per in (g0pos, g1pos)]
                outs, fences, dls = [], {}, {}

                def deadline(i, j, v):
                    dls.setdefault(i, {}).setdefault(j, []).append(v)

                def fenced16(a, key):
                    for fz in fences.pop(key, []):
                        a0 = pltpu.bitcast(_pk(a[0:RG, 0:T]) | fz, BF16)
                        a = jnp.concatenate([jnp.concatenate([a0, a[0:RG, T:]], axis=1), a[RG:]], axis=0)
                    return a

                def QK(i):
                    hh, b = units[i]
                    q = q_ref[slot(H0 + hh), b]
                    for fz in fences.pop(i, []):
                        q = jnp.concatenate([q[0:8] | fz, q[8:]], axis=0)
                    deps = dls.pop(i, None)
                    if deps:
                        parts = []
                        for j in range(NQV):
                            v = q[8 * j:8 * j + 8]
                            us = [_pk(d[r:r + 8]) for d in deps.get(j, []) for r in range(0, d.shape[0], 8)]
                            if us:
                                u = us[0]
                                for w in us[1:]:
                                    u = u | w
                                v = v | _zero_bits(u)
                            parts.append(v)
                        q = jnp.concatenate(parts, axis=0)
                    ss[i] = qk(q, slot(H0 + hh), b)

                def PV(i):
                    hh, b = units[i]
                    o, raw[i], lb = pv(ss.pop(i), slot(H0 + hh), b)
                    put_o(done, hh, b, o)
                    if i < nwin[0]:
                        for j in range(NQV):
                            deadline(i + nwin[1], j, lb[RG * j:RG * j + RG])

                def stream2(i, j, t, r0=0, nr=DQ):
                    y = _lin([(lambda pr=pr: jax.lax.dot_general(s_op(pr, i, j, r0, nr), Tm[pr](i, j, t), NT,
                                                                 preferred_element_type=F32), 1) for pr in range(2)])
                    macc[t, r0 // RG:(r0 + nr) // RG, 7 * i + j] += y.reshape(nr // RG, RG, T)

                def out_tile(c, t, y, dl, bslots=None):
                    tile = c * NT3 + t
                    if bslots is None:
                        obuf[dyn(tile)] = _bf(y.T)
                    else:
                        for d0 in range(0, D, T):
                            d1 = min(D, d0 + T)
                            v = _bf(y[d0:d1].T)
                            obuf[dyn(tile), :, d0:d1] = v
                            if d1 - d0 == T:
                                deadline(*next(bslots), _pk(v))
                    cp = pltpu.make_async_copy(obuf.at[tile], o_hbm.at[pl.ds(tile * T, T)], osem(tile))
                    cp.start()
                    outs.append(cp)
                    obuf[dyn(NTL), 0:RG, 0:T] = jnp.zeros((RG, T), obuf.dtype)
                    fences.setdefault(dl, []).append(_pk(obuf[dyn(NTL), 0:RG, 0:T]))

                def combine(c, t, toks=None, slots=None):
                    for mq in range(4):
                        for r0 in range(0, DQ, RG):
                            v = combine_rows(c, t, mq, r0, next(toks) if toks is not None else None)
                            if slots is not None:
                                deadline(*next(slots), v)
                    return base[c * NT3 + t]

                def o_cols(c, hhs):
                    return jnp.concatenate([_bf(o_tile(done, hh, r, c, TL)) for hh in hhs for r in range(rep)], axis=1)

                def o_classic(c, hhs):
                    o = o_cols(c, hhs)
                    w = jnp.concatenate([wobuf[slot(H0 + hh)] for hh in hhs], axis=1)
                    return jax.lax.dot_general(fenced16(w, ('O', c, hhs[0])), o, NT, preferred_element_type=F32)

                QK(0)
                for i in range(n):
                    if i + 1 < n:
                        QK(i + 1)
                    for t in range(TL):
                        for _ in range(gp[t].get(i, 0)):
                            stream2(*grp[t].pop(0))
                        if len(grp[t]) == 1:
                            e = grp[t].pop(0)
                            stream2(*e, 0, 80); stream2(*e, 80, 64)
                    if i in ppos:
                        c = ppos.index(i)
                        ya, yb = o_classic(c, [0, 1]), o_classic(c, [2, 3])
                        out_tile(c, TL, (base[c * NT3 + TL] + ya) + yb, pdl[c])
                        if c < 2:
                            assert not grp[1]
                            for cc, y in ((2 * c, ya), (2 * c + 1, yb)):
                                toks = iter([y[r0:r0 + 8] for r0 in range(0, D, RG)])
                                out_tile(cc, 1, combine(cc, 1, toks=toks), c1dl[cc])
                    PV(i)
                    for r0 in range(0, rep * Sq, 48):
                        if spieces:
                            prep_s(*spieces.pop(0), raw[i][r0:r0 + 8])
                        for off in (16, 32):
                            if bpieces:
                                combine_rows(*bpieces.pop(0), raw[i][r0 + off:r0 + off + 8])
                    if i == c0start:
                        assert not grp[0]
                        slots = iter([(ii, j) for ii in range(i + 2, n) for j in range(NQV)])
                        for c in range(NC):
                            e0 = i + 2 + ((c + 1) * (D // RG) - 1) // NQV
                            bs = iter([(e0 + 1 + a // 2, 3 + 6 * (a % 2)) for a in range(4)])
                            out_tile(c, 0, combine(c, 0, slots=slots), e0 + cdl, bs)
                assert not spieces and not bpieces
                c = NC - 1
                tile = c * NT3 + TL
                pre = (base[tile] + o_classic(c, [0, 1])).T
                o = fenced16(o_cols(c, [2, 3]), ('O', c, 2))
                lo = 0
                for e, d0 in enumerate(range(0, D, T)):
                    d1 = min(D, d0 + T)
                    w = jnp.concatenate([wobuf[slot(H0 + hh), d0:d1, :] for hh in (2, 3)], axis=1)
                    yb = jax.lax.dot_general(o, w, NT, preferred_element_type=F32)
                    obuf[dyn(tile), :, d0:d1] = _bf(pre[:, d0:d1] + yb)
                    if e in fsplit:
                        cols = pl.ds(lo, d1 - lo)
                        cp = pltpu.make_async_copy(obuf.at[tile, :, cols], o_hbm.at[pl.ds(tile * T, T), cols],
                                                   osem(tile + fsplit.index(e)))
                        cp.start()
                        outs.append(cp)
                        lo = d1
                assert not fences and not dls and lo == D
                with sc_('outw'):
                    for cp in outs:
                        cp.wait()

            wq0_cp(0).start()
            x_cp(0).start()
            for hh in range(1, LA):
                wq0_cp(hh).start()
            for c in range(1, NC):
                x_cp(c).start()
            for hh in range(0, LA, 2):
                wq_cp(hh).start(priority=LOW); start_kv(hh)
                wo_cp(hh).start(priority=LOW); wo_cp(hh + 1).start(priority=LOW)
                wq_cp(hh + 1).start(priority=LOW); start_kv(hh + 1)
            zs[0] = 0
            x_cp(0).wait()

            def loop_a(hh, carry):
                with sc_('wa'):
                    wq0_cp(hh).wait()
                with sc_('pa'):
                    q_classic(hh, 0, 2, wq0buf.at[hh]); q_classic(hh, 2, 2, wq0buf.at[hh])
                return carry
            jax.lax.fori_loop(0, LA, loop_a, 0)

            def loop_b(c, carry):
                with sc_('wb'):
                    x_cp(c).wait()
                with sc_('pb'):
                    toks = q_classic(0, c * CBT, CBT, wq0buf.at[0]) + q_classic(1, c * CBT, CBT, wq0buf.at[1])
                    for e, r0 in enumerate(range(0, HR, RG)):
                        t0 = (e % 4) * (CM // 4)
                        prep_x(c, r0, toks[e // 4][t0:t0 + 8])
                    for hh in range(2, LA):
                        toks += q_strassen(hh, c, wq0buf.at[hh])[2:]
                    r3 = HR // (NC - 1)
                    for e, r0 in enumerate(range(0, r3, RG)):
                        prep_x(0, (c - 1) * r3 + r0, toks[-1 - e][0:8])
                return carry
            jax.lax.fori_loop(1, NC, loop_b, 0)

            def loop_main(i, carry):
                with sc_('wait'):
                    wait_kv(2 * i); wq_cp(2 * i).wait()
                with sc_('body'):
                    main_body(2 * i)
                return carry
            jax.lax.fori_loop(0, H0 // 2, loop_main, 0)
            with sc_('wait'):
                for hh in range(H0, Hkv):
                    wait_kv(hh); wo_cp(hh).wait(); wq_cp(hh).wait()
            with sc_('tail'):
                tail()

        hbm = pl.BlockSpec(memory_space=pltpu.HBM)
        out = pl.pallas_call(
            kern,
            in_specs=[hbm] * 5,
            out_specs=hbm,
            out_shape=jax.ShapeDtypeStruct((M, D), x.dtype),
            scratch_shapes=[
                pltpu.VMEM((M, D), BF16),
                pltpu.VMEM((NB, 2, B, Sk, Dh), BF16),
                pltpu.VMEM((LA, D, W), BF16),
                pltpu.VMEM((NB, D, W), BF16),
                pltpu.VMEM((NB, D, W), BF16),
                pltpu.VMEM((NB, B, rep * Sq // 2, Dh), U32),
                pltpu.VMEM((NC, 7, HR // 2, T), U32),
                pltpu.VMEM((2, 49, DQ // 2, Dh), U32),
                pltpu.VMEM((NT3, DQ // RG, 49, RG, T), F32),
                pltpu.VMEM((NTL, D, T), F32),
                pltpu.VMEM((LA, rep, NC, CM, Dh), F32),
                pltpu.VMEM((NTL + 1, T, D), BF16),
                pltpu.SMEM((1,), jnp.int32),
                pltpu.SemaphoreType.DMA((40 + NTL + len(fsplit),)),
            ],
            compiler_params=pltpu.CompilerParams(
                vmem_limit_bytes=100 * 1024 * 1024,
                disable_bounds_checks=True, disable_semaphore_checks=True),
        )(x.reshape(M, D), k_cache, v_cache, wq, wo.T)
        return out.reshape(B, Sq, D)
    return f


pallas_standalone__gqa_block_cached__near_ridge_kernel = make()
```
